```python
import os as _os
_os.environ.setdefault("JAX_PLATFORMS", "cpu")
import jax
import jax.numpy as jnp

def _softmax(x, axis=-1):
    return jax.nn.softmax(x, axis=axis)
def _gelu(x):
    return jax.nn.gelu(x, approximate=True)
def _silu(x):
    return jax.nn.silu(x)
def _sigmoid(x):
    return jax.nn.sigmoid(x)
def _layernorm(x, axis=-1, eps=1e-5):
    m = jnp.mean(x, axis=axis, keepdims=True)
    v = jnp.var(x, axis=axis, keepdims=True)
    return (x - m) / jnp.sqrt(v + eps)
def _scatter_add(tgt, idx, src, axis=0):
    return tgt.at[idx].add(src)
def _segment_sum(src, seg, n):
    return jax.ops.segment_sum(src, seg, n)
class _Rng:
    def __init__(self, key):
        self._k = key
    def _next(self):
        self._k, sub = jax.random.split(self._k)
        return sub
    def normal(self, shape):
        return jax.random.normal(self._next(), shape, dtype=jnp.bfloat16)
    def randint(self, lo, hi, shape):
        return jax.random.randint(self._next(), shape, lo, hi, dtype=jnp.int32)
    def uniform(self, shape, lo=0.0, hi=1.0):
        return jax.random.uniform(self._next(), shape, jnp.bfloat16, lo, hi)
    def permutation(self, n):
        return jax.random.permutation(self._next(), n)


kernel_name = 'gated_mix__linear_attn_block__mixer_token_mlp__prompt'

def setup_inputs():
    _rng = _Rng(jax.random.key(int.from_bytes(__import__("os").urandom(4), "little")))
    _w = (lambda a: (lambda t: t.astype(jnp.bfloat16) if jnp.issubdtype(t.dtype, jnp.floating) else t)(jnp.asarray(a)))
    def _A_setup():
        B, S, D = 1, 2048, 512
        return {
            "x": _w((lambda *s: _rng.normal(s) * 0.05)(B, S, D)),
            "wqkv": _w((lambda *s: _rng.normal(s) * 0.8)(D, 3 * D)),
            "wo": _w((lambda *s: _rng.normal(s) * 0.05)(D, D)),
        }
    _A_in = _A_setup()

    def _B_setup():
        B, S, D, F = 1, 2048, 512, 1792
        return {
            "x": _w((lambda *s: _rng.normal(s) * 0.05)(B, S, D)),
            "w1": _w((lambda *s: _rng.normal(s) * 0.1)(S, F) * (S ** -0.5)),
            "b1": _w((lambda *s: _rng.normal(s) * 0.1)(F) * 0.02),
            "w2": _w((lambda *s: _rng.normal(s) * 0.1)(F, S) * (F ** -0.5)),
            "b2": _w((lambda *s: _rng.normal(s) * 0.1)(S) * 0.02),
        }
    _B_in = _B_setup()

    return {
        "A_x": _A_in["x"],
        "A_wqkv": _A_in["wqkv"],
        "A_wo": _A_in["wo"],
        "B_x": _B_in["x"],
        "B_w1": _B_in["w1"],
        "B_b1": _B_in["b1"],
        "B_w2": _B_in["w2"],
        "B_b2": _B_in["b2"],
        "gate_w": _w((lambda *s: _rng.normal(s) * 0.05)(512) * 16.0),
    }

def reference(A_x, A_wqkv, A_wo, B_x, B_w1, B_b1, B_w2, B_b2, gate_w):
    def _A_ref(x, wqkv, wo):
        B, S, D = x.shape
        H = 32; Dh = D // H
        qkv = (lambda x, *d: x.transpose(*d))((x @ wqkv).reshape(B, S, 3, H, Dh), 2, 0, 3, 1, 4)
        q, k, v = qkv[0], qkv[1], qkv[2]
        phi = lambda t: jnp.where(t > 0, t + 1, jnp.exp(t)) + 1e-6
        pq, pk = phi(q), phi(k)
        kv = jnp.einsum("bhsd,bhse->bhde", pk, v)
        z = jnp.einsum("bhsd->bhd", pk)
        num = jnp.einsum("bhqd,bhde->bhqe", pq, kv)
        den = jnp.einsum("bhqd,bhd->bhq", pq, z)[..., None] + 1e-6
        o = num / den
        return (lambda x, *d: x.transpose(*d))(o, 0, 2, 1, 3).reshape(B, S, D) @ wo

    def _B_ref(x, w1, b1, w2, b2):
        B, S, D = x.shape
        h = _layernorm(x, axis=-1)
        u = jnp.einsum("bsd,sf->bdf", h, w1) + b1
        u = _gelu(u)
        y = jnp.einsum("bdf,fs->bds", u, w2) + b2
        return (lambda x, *d: x.transpose(*d))(y, 0, 2, 1)

    x = A_x
    g = _sigmoid((x * gate_w).sum(-1, keepdims=True))
    a = _A_ref(x, A_wqkv, A_wo)
    b = _B_ref(x, B_w1, B_b1, B_w2, B_b2)
    return g * a + (1 - g) * b
```

```python
import functools

import jax
import jax.numpy as jnp
from jax import lax
from jax.experimental import pallas as pl
from jax.experimental.pallas import tpu as pltpu

_H = 32
_LANES = 128
_T1 = (256, 256, 512, 512, 512)
_TS2 = 512
_FC = 256


def _phi(t):
    return jnp.where(t > 0, t + 1.0, jnp.exp(t)) + 1e-6


def _gelu_tanh(x):
    c = 0.7978845608028654
    return 0.5 * x * (1.0 + jnp.tanh(c * (x + 0.044715 * (x * x * x))))


def _kernel(x_hbm, wqkv_hbm, wo_hbm, w1_hbm, w2_hbm, b1_ref, b2_ref, gw_ref,
            o_hbm,
            x_v, wqkv_v, wo_v, w1_v, w2_v, o_v,
            pq_s, pk_s, v_s, g_s, z_acc, u_acc, uact_s, m_s,
            sem_x, sem_w, sem_w1, sem_w2, sem_o,
            *, seq, d_model, dh, n_f):
    D = d_model
    S = seq
    n_groups = D // _LANES
    fc = _FC
    ts2 = _TS2
    n2 = S // ts2
    t1_sizes = _T1
    t1_offs = [sum(t1_sizes[:i]) for i in range(len(t1_sizes))]
    n1 = len(t1_sizes)

    def x_cp(t):
        r = pl.ds(t1_offs[t], t1_sizes[t])
        return pltpu.make_async_copy(x_hbm.at[r, :], x_v.at[r, :], sem_x.at[t])

    def w1_cp(t):
        r = pl.ds(t1_offs[t], t1_sizes[t])
        return pltpu.make_async_copy(w1_hbm.at[r, :], w1_v.at[r, :], sem_w1.at[t])

    def w2_cp(t):
        c = pl.ds(t * ts2, ts2)
        return pltpu.make_async_copy(w2_hbm.at[:, c], w2_v.at[:, c], sem_w2.at[t])

    def o_cp(t):
        r = pl.ds(t * ts2, ts2)
        return pltpu.make_async_copy(o_v.at[r, :], o_hbm.at[r, :], sem_o.at[t])

    def wqkv_cp(j):
        c = pl.ds(j * D, D)
        return pltpu.make_async_copy(wqkv_hbm.at[:, c], wqkv_v.at[:, c], sem_w.at[j])

    wo_cp = pltpu.make_async_copy(wo_hbm, wo_v, sem_w.at[3])

    x_cp(0).start()
    for j in range(3):
        wqkv_cp(j).start()
    w1_cp(0).start()

    z_acc[...] = jnp.zeros_like(z_acc)
    u_acc[...] = jnp.zeros_like(u_acc)
    gw = gw_ref[...].astype(jnp.float32).reshape(1, D)
    b1r = b1_ref[...].astype(jnp.float32).reshape(1, b1_ref.shape[0])
    b2r = b2_ref[...].astype(jnp.float32).reshape(1, S)


    r_ = lax.broadcasted_iota(jnp.int32, (_LANES, _LANES), 0) // dh
    c_ = lax.broadcasted_iota(jnp.int32, (_LANES, _LANES), 1) // dh
    mask = r_ == c_

    def mid_group(g):
        sl = slice(g * _LANES, (g + 1) * _LANES)
        kv = lax.dot_general(pk_s[:, sl], v_s[:, sl], (((0,), (0,)), ((), ())),
                             preferred_element_type=jnp.float32)
        kvg = jnp.where(mask, kv, 0.0).astype(jnp.bfloat16)
        m_s[sl, :] = jnp.dot(kvg, wo_v[sl, :],
                             preferred_element_type=jnp.float32).astype(jnp.bfloat16)
        zg = z_acc[:, sl]
        zcol = jnp.broadcast_to(zg, (_LANES, _LANES)).T
        zmat = jnp.where(mask, zcol, 0.0).astype(jnp.bfloat16)
        pqg = pq_s[:, sl]
        den = jnp.dot(pqg, zmat, preferred_element_type=jnp.float32) + 1e-6
        pq_s[:, sl] = (pqg.astype(jnp.float32) / den).astype(jnp.bfloat16)

    for t in range(n1):
        rows = pl.ds(t1_offs[t], t1_sizes[t])
        x_cp(t).wait()
        if t == 0:
            for t2 in range(1, n1):
                x_cp(t2).start()
                w1_cp(t2).start()
            wo_cp.start()
            for t2 in range(n2):
                w2_cp(t2).start()
        xt = x_v[rows, :]
        xf = xt.astype(jnp.float32)

        if t == 0:
            wqkv_cp(0).wait()
        q = jnp.dot(xt, wqkv_v[:, 0:D], preferred_element_type=jnp.float32)
        pq_s[rows, :] = _phi(q).astype(jnp.bfloat16)
        gl = jnp.sum(xf * gw, axis=-1, keepdims=True)
        g_s[rows, :] = jax.nn.sigmoid(gl)
        m = jnp.mean(xf, axis=-1, keepdims=True)
        xc = xf - m
        var = jnp.mean(xc * xc, axis=-1, keepdims=True)
        h = xc * lax.rsqrt(var + 1e-5)
        hT = h.T.astype(jnp.bfloat16)

        if t == 0:
            wqkv_cp(1).wait()
        k = jnp.dot(xt, wqkv_v[:, D:2 * D], preferred_element_type=jnp.float32)
        pk = _phi(k)
        z_acc[...] += jnp.sum(pk, axis=0, keepdims=True)
        pk_s[rows, :] = pk.astype(jnp.bfloat16)
        if t == 0:
            wqkv_cp(2).wait()
        v = jnp.dot(xt, wqkv_v[:, 2 * D:3 * D], preferred_element_type=jnp.float32)
        v_s[rows, :] = v.astype(jnp.bfloat16)

        w1_cp(t).wait()
        if t < n1 - 1:
            u_acc[...] += jnp.dot(hT, w1_v[rows, :],
                                  preferred_element_type=jnp.float32)
        else:
            for c in range(n_f):
                cs = slice(c * fc, (c + 1) * fc)
                u = u_acc[:, cs] + jnp.dot(hT, w1_v[rows, cs],
                                           preferred_element_type=jnp.float32)
                u = u + b1r[:, cs]
                uact_s[:, cs] = _gelu_tanh(u).astype(jnp.bfloat16)
                if c == 0:
                    wo_cp.wait()
                if c < n_groups:
                    mid_group(c)

    for t in range(n2):
        rows = pl.ds(t * ts2, ts2)
        w2_cp(t).wait()
        y = jnp.dot(uact_s[...], w2_v[:, rows],
                    preferred_element_type=jnp.float32)
        y = y + b2r[:, t * ts2:(t + 1) * ts2]
        bt = y.T
        a = jnp.dot(pq_s[rows, :], m_s[...], preferred_element_type=jnp.float32)
        gt = g_s[rows, :]
        o_v[rows, :] = (gt * a + (1.0 - gt) * bt).astype(o_v.dtype)
        o_cp(t).start()

    for t in range(n2):
        o_cp(t).wait()


@jax.jit
def pallas_gated_mix__linear_attn_block__mixer_token_mlp__prompt_kernel(
    A_x: jax.Array,
    A_wqkv: jax.Array,
    A_wo: jax.Array,
    B_x: jax.Array,
    B_w1: jax.Array,
    B_b1: jax.Array,
    B_w2: jax.Array,
    B_b2: jax.Array,
    gate_w: jax.Array,
):
    Bsz, S, D = A_x.shape
    assert Bsz == 1
    F = B_w1.shape[1]
    dh = D // _H
    n_f = F // _FC
    n1, n2 = len(_T1), S // _TS2

    x = A_x.reshape(S, D)

    kern = functools.partial(_kernel, seq=S, d_model=D, dh=dh, n_f=n_f)
    any_spec = pl.BlockSpec(memory_space=pl.ANY)
    vmem_spec = pl.BlockSpec(memory_space=pltpu.VMEM)

    out = pl.pallas_call(
        kern,
        in_specs=[any_spec, any_spec, any_spec, any_spec, any_spec,
                  vmem_spec, vmem_spec, vmem_spec],
        out_specs=any_spec,
        out_shape=jax.ShapeDtypeStruct((S, D), A_x.dtype),
        scratch_shapes=[
            pltpu.VMEM((S, D), jnp.bfloat16),
            pltpu.VMEM((D, 3 * D), jnp.bfloat16),
            pltpu.VMEM((D, D), jnp.bfloat16),
            pltpu.VMEM((S, F), jnp.bfloat16),
            pltpu.VMEM((F, S), jnp.bfloat16),
            pltpu.VMEM((S, D), jnp.bfloat16),
            pltpu.VMEM((S, D), jnp.bfloat16),
            pltpu.VMEM((S, D), jnp.bfloat16),
            pltpu.VMEM((S, D), jnp.bfloat16),
            pltpu.VMEM((S, 1), jnp.float32),
            pltpu.VMEM((1, D), jnp.float32),
            pltpu.VMEM((D, F), jnp.float32),
            pltpu.VMEM((D, F), jnp.bfloat16),
            pltpu.VMEM((D, D), jnp.bfloat16),
            pltpu.SemaphoreType.DMA((n1,)),
            pltpu.SemaphoreType.DMA((4,)),
            pltpu.SemaphoreType.DMA((n1,)),
            pltpu.SemaphoreType.DMA((n2,)),
            pltpu.SemaphoreType.DMA((n2,)),
        ],
        compiler_params=pltpu.CompilerParams(
            vmem_limit_bytes=100 * 1024 * 1024,
        ),
    )(x, A_wqkv, A_wo, B_w1, B_w2, B_b1, B_b2, gate_w)
    return out.reshape(Bsz, S, D)
```
